```python
import jax
import jax.numpy as jnp

def _softmax(x, axis=-1):
    return jax.nn.softmax(x, axis=axis)
def _gelu(x):
    return jax.nn.gelu(x, approximate=True)
def _silu(x):
    return jax.nn.silu(x)
def _sigmoid(x):
    return jax.nn.sigmoid(x)
def _layernorm(x, axis=-1, eps=1e-5):
    m = jnp.mean(x, axis=axis, keepdims=True)
    v = jnp.var(x, axis=axis, keepdims=True)
    return (x - m) / jnp.sqrt(v + eps)
def _scatter_add(tgt, idx, src, axis=0):
    return tgt.at[idx].add(src)
def _segment_sum(src, seg, n):
    return jax.ops.segment_sum(src, seg, n)
class _Rng:
    def __init__(self, key):
        self._k = key
    def _next(self):
        self._k, sub = jax.random.split(self._k)
        return sub
    def normal(self, shape):
        return jax.random.normal(self._next(), shape, dtype=jnp.bfloat16)
    def randint(self, lo, hi, shape):
        return jax.random.randint(self._next(), shape, lo, hi, dtype=jnp.int32)
    def uniform(self, shape, lo=0.0, hi=1.0):
        return jax.random.uniform(self._next(), shape, jnp.bfloat16, lo, hi)
    def permutation(self, n):
        return jax.random.permutation(self._next(), n)


kernel_name = 'sequential_preLN__sliding_block_cached__glu_gated_swiglu__decode'

def setup_inputs():
    _rng = _Rng(jax.random.key(int.from_bytes(__import__("os").urandom(4), "little")))
    _w = (lambda a: (lambda t: t.astype(jnp.bfloat16) if jnp.issubdtype(t.dtype, jnp.floating) else t)(jnp.asarray(a)))
    def _A_setup():
        B, Sq, D = 1, 1, 640
        Hq, Hkv, Sk, Dh = 32, 32, 32768, 192
        assert Hq % Hkv == 0, (Hq, Hkv)
        return {
            "x": _w((lambda *s: _rng.normal(s) * 0.05)(B, Sq, D)),
            "k_cache": _w((lambda *s: _rng.normal(s) * 0.05)(B, Hkv, Sk, Dh)),
            "v_cache": _w((lambda *s: _rng.normal(s) * 0.05)(B, Hkv, Sk, Dh)),
            "wq": _w((lambda *s: _rng.normal(s) * 0.05)(D, Hq * Dh) * (D ** -0.5)),
            "wo": _w((lambda *s: _rng.normal(s) * 0.05)(Hq * Dh, D) * ((Hq * Dh) ** -0.5)),
        }
    _A_in = _A_setup()

    def _B_setup():
        B, S, D, F = 1, 1, 640, 1536
        return {
            "x": _w((lambda *s: _rng.normal(s) * 0.05)(B, S, D)),
            "w1": _w((lambda *s: _rng.normal(s) * 0.05)(D, F) * (2.0 / D) ** 0.5),
            "w3": _w((lambda *s: _rng.normal(s) * 0.05)(D, F) * (2.0 / D) ** 0.5),
            "w2": _w((lambda *s: _rng.normal(s) * 0.05)(F, D) * (2.0 / F) ** 0.5),
        }
    _B_in = _B_setup()

    return {
        "A_x": _A_in["x"],
        "A_k_cache": _A_in["k_cache"],
        "A_v_cache": _A_in["v_cache"],
        "A_wq": _A_in["wq"],
        "A_wo": _A_in["wo"],
        "B_x": _B_in["x"],
        "B_w1": _B_in["w1"],
        "B_w3": _B_in["w3"],
        "B_w2": _B_in["w2"],
    }

def reference(A_x, A_k_cache, A_v_cache, A_wq, A_wo, B_x, B_w1, B_w3, B_w2):
    def _A_ref(x, k_cache, v_cache, wq, wo):
        B, Sq, D = x.shape
        Hq, Dh = 32, 192
        Hkv, Sk = k_cache.shape[1], k_cache.shape[2]
        W = min(4096, max(256, Sk // 4))
        rep = Hq // Hkv
        q = (lambda x, *d: x.transpose(*d))((x @ wq).reshape(B, Sq, Hq, Dh), 0, 2, 1, 3)
        k = jnp.repeat(k_cache[:, :, Sk - W:, :], rep, axis=1)
        v = jnp.repeat(v_cache[:, :, Sk - W:, :], rep, axis=1)
        scores = jnp.einsum("bhqd,bhkd->bhqk", q, k) * (Dh ** -0.5)
        p = _softmax(scores, axis=-1)
        o = jnp.einsum("bhqk,bhkd->bhqd", p, v)
        return (lambda x, *d: x.transpose(*d))(o, 0, 2, 1, 3).reshape(B, Sq, Hq * Dh) @ wo

    def _B_ref(x, w1, w3, w2):
        gate = jnp.einsum("bsd,df->bsf", x, w1)
        up = jnp.einsum("bsd,df->bsf", x, w3)
        h = _silu(gate) * up
        out = jnp.einsum("bsf,fd->bsd", h, w2)
        return out

    x = A_x
    h = x + _A_ref(_layernorm(x, axis=-1), A_k_cache, A_v_cache, A_wq, A_wo)
    h2 = h + _B_ref(_layernorm(h, axis=-1), B_w1, B_w3, B_w2)
    return h2
```

```python
import jax
import jax.numpy as jnp
import numpy as np
from jax import lax
import jax.experimental.pallas as pl
import jax.experimental.pallas.tpu as pltpu

H, DH, SK, D, F = 32, 192, 32768, 640, 1536
W = min(4096, max(256, SK // 4))
BF = jnp.bfloat16
F32 = jnp.float32


def _bf16_round(v):
    u = int(np.float32(v).view(np.uint32))
    u = (u + 0x7FFF + ((u >> 16) & 1)) & 0xFFFF0000
    return float(np.uint32(u).view(np.float32))


SCALE = _bf16_round(DH ** -0.5)
EPS = _bf16_round(1e-5)


def _r(x):
    return x.astype(BF).astype(F32)


def _layernorm(x32):
    m = jnp.mean(x32, axis=-1, keepdims=True)
    c = x32 - m
    v = jnp.mean(c * c, axis=-1, keepdims=True)
    num = _r(x32 - _r(m))
    den = _r(jnp.sqrt(_r(_r(v) + EPS)))
    return (num / den).astype(BF)


RING = 5
GQ = 5
NQ = 2
W2_STARTS = ((0, 384, 768, 1152), (128, 512, 896, 1280), (256, 640, 1024, 1408))
VPU_ROWS = (16, 16, 16)
N_MXU, N_VPU = len(W2_STARTS), sum(VPU_ROWS)
W2_CHUNKS = [[(r, 128) for r in starts] for starts in W2_STARTS[:-1]]
W2_CHUNKS.append([(r, 128 - N_VPU) for r in W2_STARTS[-1]])
W2_CHUNKS += [[(r + 128 - N_VPU + sum(VPU_ROWS[:i]), n) for r in W2_STARTS[-1]] for i, n in enumerate(VPU_ROWS)]


def _alternate(a, b):
    assert len(a) == len(b)
    return [job for x, y in zip(a, b) for job in (x + (0,), y + (1,))]


def _issue(jobs, sem):
    for src, dst, idx, thread in jobs:
        idx = tuple(pl.ds(start, size) for start, size in idx)
        pltpu.make_async_copy(src.at[idx], dst.at[idx], sem).start(priority=thread)


def _wait(ref, sem):
    pltpu.make_async_copy(ref, ref, sem).wait()


def _kernel(x_hbm, kt_hbm, vt_hbm, wq_hbm, wo_hbm, w1_hbm, w3_hbm, w2_hbm, o_hbm,
            x_v, wq_v, q_v, kv_v, wo_v, w13_v, w2_v, hcol_v, acc_v, o_v, sem_w, sem_kv, sem_w13, sem_w2, sem_o):

    def issue_head(h, slot, part=0, parts=1):
        ksrc = kt_hbm.at[h, :, pl.ds(SK - W, W)]
        vsrc = vt_hbm.at[h, :, pl.ds(SK - W, W)]
        pieces = [((r, 32), (c, 512)) for c in range(0, W, 512) for r in range(0, DH, 32)]
        jobs = _alternate([(ksrc, kv_v.at[slot, 0], p) for p in pieces], [(vsrc, kv_v.at[slot, 1], p) for p in pieces])
        _issue(jobs[part * len(jobs) // parts:(part + 1) * len(jobs) // parts], sem_kv.at[slot])

    def issue_w2(c):
        rows, threads = (16, (0, 0, 1, 1)) if c < N_MXU - 1 else (8, (0, 1))
        segs = W2_CHUNKS[c]
        jobs = [(w2_hbm, w2_v, ((r0 + r, rows),)) for r in range(0, segs[0][1], rows) for r0, _ in segs]
        _issue([j + (threads[i % len(threads)],) for i, j in enumerate(jobs)], sem_w2.at[c])

    wq_jobs = [(wq_hbm, wq_v, ((a, min(3, GQ - a)), (r, 8), (c, 512)))
               for r in range(0, D // GQ, 8) for c in range(0, H * DH, 512) for a in range(0, GQ, 3)]
    wo_jobs = [(wo_hbm, wo_v, ((a + r, 16),)) for r in range(0, H * DH // 8, 16) for a in range(0, H * DH, H * DH // 8)]
    jobs = _alternate(wq_jobs[:len(wq_jobs) // 2], wq_jobs[len(wq_jobs) // 2:])
    jobs += [j + ((i // 2) % 2,) for i, j in enumerate(wo_jobs)]
    _issue(jobs[:2], sem_w)
    pltpu.make_async_copy(x_hbm, x_v, sem_w).start()
    _issue(jobs[2:], sem_w)

    def first_heads(h, carry):
        issue_head(h, h)
        return carry

    lax.fori_loop(0, RING - 1, first_heads, 0)
    _wait(x_v, sem_w)
    _wait(wq_v, sem_w)
    _wait(wo_v, sem_w)
    x32 = x_v[...].astype(F32)
    lnx = jnp.broadcast_to(_layernorm(x32), (8, D))
    hq = H // NQ
    for c in range(NQ):
        wq_c = wq_v[:, :, c * hq * DH:(c + 1) * hq * DH].reshape(D, hq * DH)
        qc = jnp.dot(lnx, wq_c, preferred_element_type=F32)
        for j in range(hq):
            q_v[c * hq + j] = qc[:, j * DH:(j + 1) * DH]
        issue_head(RING - 1, RING - 1, c, NQ)

    def head_compute(h, slot, attn):
        _wait(kv_v.at[slot], sem_kv.at[slot])
        qh = q_v[h].astype(BF)
        s = jnp.dot(qh, kv_v[slot, 0], preferred_element_type=F32)
        s = _r(_r(s) * SCALE)
        m = jnp.max(s, axis=-1, keepdims=True)
        e = _r(jnp.exp(_r(s - m)))
        l = _r(jnp.sum(e, axis=-1, keepdims=True))
        p = (e / l).astype(BF)
        o = lax.dot_general(p, kv_v[slot, 1], (((1,), (1,)), ((), ())), preferred_element_type=F32)
        row = h * DH if isinstance(h, int) else pl.multiple_of(h * DH, DH)
        return attn + jnp.dot(o.astype(BF), wo_v[pl.ds(row, DH), :], preferred_element_type=F32)

    def head(h, attn):
        slot = h % RING
        attn = head_compute(h, slot, attn)
        issue_head(h + RING, slot)
        return attn

    attn = lax.fori_loop(0, H - RING, head, jnp.zeros((8, D), F32))

    pieces = [((a + r, 8),) for r in range(0, D // 4, 8) for a in range(0, D, D // 4)]
    w13_jobs = _alternate([(w1_hbm, w13_v.at[0], p) for p in pieces], [(w3_hbm, w13_v.at[1], p) for p in pieces])
    for i, h in enumerate(range(H - RING, H)):
        attn = head_compute(h, h % RING, attn)
        if i < RING - 1:
            _issue(w13_jobs[i * len(w13_jobs) // (RING - 1):(i + 1) * len(w13_jobs) // (RING - 1)], sem_w13)
    hres = _r(x32 + _r(attn))
    lnh = _layernorm(hres)

    issue_w2(0)
    _wait(w13_v.at[0], sem_w13)
    issue_w2(1)
    _wait(w13_v.at[1], sem_w13)
    gate = _r(jnp.dot(lnh, w13_v[0], preferred_element_type=F32))
    up = _r(jnp.dot(lnh, w13_v[1], preferred_element_type=F32))
    hm = (_r(gate * _r(jax.nn.sigmoid(gate))) * up).astype(BF)
    for i, r0 in enumerate(W2_STARTS[-1]):
        col = jnp.broadcast_to(hm[0:1, r0:r0 + 128].astype(F32), (128, 128)).T
        hcol_v[i] = col[128 - N_VPU:]
    late = len(W2_CHUNKS) - 2
    for k in range(late):
        issue_w2(2 + k)
        _wait(w2_v.at[pl.ds(0, 512 // late)], sem_w2.at[0])

    out = None
    for c in range(N_MXU):
        if c > 0:
            _wait(w2_v.at[pl.ds(0, sum(n for _, n in W2_CHUNKS[c]))], sem_w2.at[c])
        for r0, n in W2_CHUNKS[c]:
            part = jnp.dot(hm[:, r0:r0 + n], w2_v[r0:r0 + n, :], preferred_element_type=F32)
            out = part if out is None else out + part
    acc_v[...] = jnp.where(lax.broadcasted_iota(jnp.int32, (8, D), 0) == 0, out, 0.0)
    cols = []
    for c in range(N_MXU, len(W2_CHUNKS)):
        _wait(w2_v.at[pl.ds(0, sum(n for _, n in W2_CHUNKS[c]))], sem_w2.at[c])
        k0 = sum(VPU_ROWS[:c - N_MXU])
        for j in range(0, D, 128):
            terms = [acc_v[:, j:j + 128]]
            for i, (r0, n) in enumerate(W2_CHUNKS[c]):
                prod = w2_v[r0:r0 + n, j:j + 128].astype(F32) * hcol_v[i, k0:k0 + n]
                terms += [prod[k:k + 8] for k in range(0, n, 8)]
            while len(terms) > 1:
                terms = [sum(terms[k + 1:k + 2], terms[k]) for k in range(0, len(terms), 2)]
            if c < len(W2_CHUNKS) - 1:
                acc_v[:, j:j + 128] = terms[0]
            else:
                cols.append(jnp.sum(terms[0], axis=0, keepdims=True))
    o_v[...] = (hres[0:1] + _r(jnp.concatenate(cols, axis=1))).astype(o_v.dtype)
    out_copy = pltpu.make_async_copy(o_v, o_hbm, sem_o)
    out_copy.start()
    out_copy.wait()


@jax.jit
def pallas_sequential_preLN__sliding_block_cached__glu_gated_swiglu__decode_kernel(
        A_x, A_k_cache, A_v_cache, A_wq, A_wo, B_x, B_w1, B_w3, B_w2):
    del B_x
    kt = jnp.swapaxes(A_k_cache.reshape(H, SK, DH), 1, 2)
    vt = jnp.swapaxes(A_v_cache.reshape(H, SK, DH), 1, 2)
    dma = pltpu.SemaphoreType.DMA
    out = pl.pallas_call(
        _kernel,
        out_shape=jax.ShapeDtypeStruct((1, D), A_x.dtype),
        in_specs=[pl.BlockSpec(memory_space=pl.ANY)] * 8,
        out_specs=pl.BlockSpec(memory_space=pl.ANY),
        scratch_shapes=[
            pltpu.VMEM((1, D), BF),
            pltpu.VMEM((GQ, D // GQ, H * DH), BF),
            pltpu.VMEM((H, 8, DH), F32),
            pltpu.VMEM((RING, 2, DH, W), BF),
            pltpu.VMEM((H * DH, D), BF),
            pltpu.VMEM((2, D, F), BF),
            pltpu.VMEM((F, D), BF),
            pltpu.VMEM((len(W2_STARTS[-1]), N_VPU, 128), F32),
            pltpu.VMEM((8, D), F32),
            pltpu.VMEM((1, D), BF),
            dma(()), dma((RING,)), dma(()), dma((len(W2_CHUNKS),)), dma(()),
        ],
        compiler_params=pltpu.CompilerParams(vmem_limit_bytes=64 * 1024 * 1024, disable_bounds_checks=True,
                                             disable_semaphore_checks=True),
    )(A_x.reshape(1, D), kt, vt, A_wq.reshape(GQ, D // GQ, H * DH), A_wo, B_w1, B_w3, B_w2)
    return out.reshape(1, 1, D)
```

```python
import jax
import jax.numpy as jnp
import numpy as np
from jax import lax
import jax.experimental.pallas as pl
import jax.experimental.pallas.tpu as pltpu

H, DH, SK, D, F = 32, 192, 32768, 640, 1536
W = min(4096, max(256, SK // 4))
BF = jnp.bfloat16
F32 = jnp.float32


def _bf16_round(v):
    u = int(np.float32(v).view(np.uint32))
    u = (u + 0x7FFF + ((u >> 16) & 1)) & 0xFFFF0000
    return float(np.uint32(u).view(np.float32))


SCALE = _bf16_round(DH ** -0.5)
EPS = _bf16_round(1e-5)


def _r(x):
    return x.astype(BF).astype(F32)


def _layernorm(x32):
    m = jnp.mean(x32, axis=-1, keepdims=True)
    c = x32 - m
    v = jnp.mean(c * c, axis=-1, keepdims=True)
    num = _r(x32 - _r(m))
    den = _r(jnp.sqrt(_r(_r(v) + EPS)))
    return (num / den).astype(BF)


RING = 5
GQ = 5
NQ = 2
W2_STARTS = ((0, 384, 768, 1152), (128, 512, 896, 1280), (256, 640, 1024, 1408))
VPU_ROWS = (16, 16, 16)
N_MXU, N_VPU = len(W2_STARTS), sum(VPU_ROWS)
W2_CHUNKS = [[(r, 128) for r in starts] for starts in W2_STARTS[:-1]]
W2_CHUNKS.append([(r, 128 - N_VPU) for r in W2_STARTS[-1]])
W2_CHUNKS += [[(r + 128 - N_VPU + sum(VPU_ROWS[:i]), n) for r in W2_STARTS[-1]] for i, n in enumerate(VPU_ROWS)]
assert len(W2_CHUNKS) == 2 + len(W2_CHUNKS[0])


def _alternate(a, b):
    assert len(a) == len(b)
    return [job for x, y in zip(a, b) for job in (x + (0,), y + (1,))]


def _issue(jobs, sem):
    for src, dst, idx, thread in jobs:
        idx = tuple(pl.ds(start, size) for start, size in idx)
        pltpu.make_async_copy(src.at[idx], dst.at[idx], sem).start(priority=thread)


def _wait(ref, sem):
    pltpu.make_async_copy(ref, ref, sem).wait()


def _body(x_hbm, kt_hbm, vt_hbm, wq_hbm, wo_hbm, w1_hbm, w3_hbm, w2_hbm, o_hbm,
          x_v, wq_v, q_v, kv_v, wo_v, w13_v, w2_v, hcol_v, acc_v, o_v, sem_o, sem_w, sem_kv, sem_w13, sem_w2):

    def issue_head(h, slot, part=0, parts=1):
        ksrc = kt_hbm.at[h, :, pl.ds(SK - W, W)]
        vsrc = vt_hbm.at[h, :, pl.ds(SK - W, W)]
        pieces = [((r, 32), (c, 512)) for c in range(0, W, 512) for r in range(0, DH, 32)]
        jobs = _alternate([(ksrc, kv_v.at[slot, 0], p) for p in pieces], [(vsrc, kv_v.at[slot, 1], p) for p in pieces])
        _issue(jobs[part * len(jobs) // parts:(part + 1) * len(jobs) // parts], sem_kv.at[slot])

    def issue_w2(c):
        rows, threads = (16, (0, 0, 1, 1)) if c < N_MXU - 1 else (8, (0, 1))
        segs = W2_CHUNKS[c]
        jobs = [(w2_hbm, w2_v, ((r0 + r, rows),)) for r in range(0, segs[0][1], rows) for r0, _ in segs]
        _issue([j + (threads[i % len(threads)],) for i, j in enumerate(jobs)], sem_w2.at[c])

    def wait_w2(c):
        for r0, n in W2_CHUNKS[c]:
            _wait(w2_v.at[pl.ds(r0, n)], sem_w2.at[c])

    wq_jobs = [(wq_hbm, wq_v, ((a, min(2, GQ - a)), (r, 8), (c, 512)))
               for r in range(0, D // GQ, 8) for c in range(0, H * DH, 512) for a in range(0, GQ, 2)]
    wo_jobs = [(wo_hbm, wo_v, ((a + r, 16),)) for r in range(0, H * DH // 8, 16) for a in range(0, H * DH, H * DH // 8)]
    jobs = _alternate(wq_jobs[:len(wq_jobs) // 2], wq_jobs[len(wq_jobs) // 2:])
    jobs += [j + ((i // 2) % 2,) for i, j in enumerate(wo_jobs)]
    _issue(jobs[:2], sem_w)
    pltpu.make_async_copy(x_hbm, x_v, sem_w).start()
    _issue(jobs[2:], sem_w)

    def first_heads(h, carry):
        issue_head(h, h)
        return carry

    lax.fori_loop(0, RING - 1, first_heads, 0)
    _wait(x_v, sem_w)
    _wait(wq_v, sem_w)
    _wait(wo_v, sem_w)
    x32 = x_v[...].astype(F32)
    lnx = jnp.broadcast_to(_layernorm(x32), (8, D))
    hq = H // NQ
    for c in range(NQ):
        wq_c = wq_v[:, :, c * hq * DH:(c + 1) * hq * DH].reshape(D, hq * DH)
        qc = jnp.dot(lnx, wq_c, preferred_element_type=F32)
        for j in range(hq):
            q_v[c * hq + j] = qc[:, j * DH:(j + 1) * DH]
        issue_head(RING - 1, RING - 1, c, NQ)

    def head_compute(h, slot, attn):
        _wait(kv_v.at[slot], sem_kv.at[slot])
        qh = q_v[h].astype(BF)
        s = jnp.dot(qh, kv_v[slot, 0], preferred_element_type=F32)
        s = _r(_r(s) * SCALE)
        m = jnp.max(s, axis=-1, keepdims=True)
        e = _r(jnp.exp(_r(s - m)))
        l = _r(jnp.sum(e, axis=-1, keepdims=True))
        p = (e / l).astype(BF)
        o = lax.dot_general(p, kv_v[slot, 1], (((1,), (1,)), ((), ())), preferred_element_type=F32)
        row = h * DH if isinstance(h, int) else pl.multiple_of(h * DH, DH)
        return attn + jnp.dot(o.astype(BF), wo_v[pl.ds(row, DH), :], preferred_element_type=F32)

    def head(h, attn):
        slot = h % RING
        attn = head_compute(h, slot, attn)
        issue_head(h + RING, slot)
        return attn

    attn = lax.fori_loop(0, H - RING, head, jnp.zeros((8, D), F32))

    pieces = [((a + r, 8),) for r in range(0, D // 4, 8) for a in range(0, D, D // 4)]
    w13_jobs = _alternate([(w1_hbm, w13_v.at[0], p) for p in pieces], [(w3_hbm, w13_v.at[1], p) for p in pieces])
    for i, h in enumerate(range(H - RING, H)):
        attn = head_compute(h, h % RING, attn)
        if i < RING - 1:
            _issue(w13_jobs[i * len(w13_jobs) // (RING - 1):(i + 1) * len(w13_jobs) // (RING - 1)], sem_w13)
    hres = _r(x32 + _r(attn))
    lnh = _layernorm(hres)

    issue_w2(0)
    _wait(w13_v.at[0], sem_w13)
    issue_w2(1)
    _wait(w13_v.at[1], sem_w13)
    gate = _r(jnp.dot(lnh, w13_v[0], preferred_element_type=F32))
    up = _r(jnp.dot(lnh, w13_v[1], preferred_element_type=F32))
    hm = (_r(gate * _r(jax.nn.sigmoid(gate))) * up).astype(BF)
    for i, r0 in enumerate(W2_STARTS[-1]):
        col = jnp.broadcast_to(hm[0:1, r0:r0 + 128].astype(F32), (128, 128)).T
        hcol_v[i] = col[128 - N_VPU:]
    for k, (r0, n) in enumerate(W2_CHUNKS[0]):
        issue_w2(2 + k)
        _wait(w2_v.at[pl.ds(r0, n)], sem_w2.at[0])

    out = None
    for c in range(N_MXU):
        if c > 0:
            wait_w2(c)
        for r0, n in W2_CHUNKS[c]:
            part = jnp.dot(hm[:, r0:r0 + n], w2_v[r0:r0 + n, :], preferred_element_type=F32)
            out = part if out is None else out + part
    acc_v[...] = jnp.where(lax.broadcasted_iota(jnp.int32, (8, D), 0) == 0, out, 0.0)
    cols = []
    for c in range(N_MXU, len(W2_CHUNKS)):
        wait_w2(c)
        k0 = sum(VPU_ROWS[:c - N_MXU])
        for j in range(0, D, 128):
            terms = [acc_v[:, j:j + 128]]
            for i, (r0, n) in enumerate(W2_CHUNKS[c]):
                prod = w2_v[r0:r0 + n, j:j + 128].astype(F32) * hcol_v[i, k0:k0 + n]
                terms += [prod[k:k + 8] for k in range(0, n, 8)]
            while len(terms) > 1:
                terms = [sum(terms[k + 1:k + 2], terms[k]) for k in range(0, len(terms), 2)]
            if c < len(W2_CHUNKS) - 1:
                acc_v[:, j:j + 128] = terms[0]
            else:
                cols.append(jnp.sum(terms[0], axis=0, keepdims=True))
    o_v[...] = (hres[0:1] + _r(jnp.concatenate(cols, axis=1))).astype(o_v.dtype)
    pltpu.make_async_copy(o_v, o_hbm, sem_o).start()


def _kernel(*refs):
    o_hbm, o_v, sem_o = refs[8], refs[-2], refs[-1]
    dma = pltpu.SemaphoreType.DMA
    pl.run_scoped(lambda *sems: _body(*refs, *sems), dma(()), dma((RING,)), dma(()), dma((len(W2_CHUNKS),)))
    pltpu.make_async_copy(o_v, o_hbm, sem_o).wait()


@jax.jit
def pallas_sequential_preLN__sliding_block_cached__glu_gated_swiglu__decode_kernel(
        A_x, A_k_cache, A_v_cache, A_wq, A_wo, B_x, B_w1, B_w3, B_w2):
    del B_x
    kt = jnp.swapaxes(A_k_cache.reshape(H, SK, DH), 1, 2)
    vt = jnp.swapaxes(A_v_cache.reshape(H, SK, DH), 1, 2)
    out = pl.pallas_call(
        _kernel,
        out_shape=jax.ShapeDtypeStruct((1, D), A_x.dtype),
        in_specs=[pl.BlockSpec(memory_space=pl.ANY)] * 8,
        out_specs=pl.BlockSpec(memory_space=pl.ANY),
        scratch_shapes=[
            pltpu.VMEM((1, D), BF),
            pltpu.VMEM((GQ, D // GQ, H * DH), BF),
            pltpu.VMEM((H, 8, DH), F32),
            pltpu.VMEM((RING, 2, DH, W), BF),
            pltpu.VMEM((H * DH, D), BF),
            pltpu.VMEM((2, D, F), BF),
            pltpu.VMEM((F, D), BF),
            pltpu.VMEM((len(W2_STARTS[-1]), N_VPU, 128), F32),
            pltpu.VMEM((8, D), F32),
            pltpu.VMEM((1, D), BF),
            pltpu.SemaphoreType.DMA(()),
        ],
        compiler_params=pltpu.CompilerParams(vmem_limit_bytes=64 * 1024 * 1024),
    )(A_x.reshape(1, D), kt, vt, A_wq.reshape(GQ, D // GQ, H * DH), A_wo, B_w1, B_w3, B_w2)
    return out.reshape(1, 1, D)
```
